```python
import os as _os
_os.environ.setdefault("JAX_PLATFORMS", "cpu")
import jax
import jax.numpy as jnp

def _softmax(x, axis=-1):
    return jax.nn.softmax(x, axis=axis)
def _gelu(x):
    return jax.nn.gelu(x, approximate=True)
def _silu(x):
    return jax.nn.silu(x)
def _sigmoid(x):
    return jax.nn.sigmoid(x)
def _layernorm(x, axis=-1, eps=1e-5):
    m = jnp.mean(x, axis=axis, keepdims=True)
    v = jnp.var(x, axis=axis, keepdims=True)
    return (x - m) / jnp.sqrt(v + eps)
def _scatter_add(tgt, idx, src, axis=0):
    return tgt.at[idx].add(src)
def _segment_sum(src, seg, n):
    return jax.ops.segment_sum(src, seg, n)
class _Rng:
    def __init__(self, key):
        self._k = key
    def _next(self):
        self._k, sub = jax.random.split(self._k)
        return sub
    def normal(self, shape):
        return jax.random.normal(self._next(), shape, dtype=jnp.bfloat16)
    def randint(self, lo, hi, shape):
        return jax.random.randint(self._next(), shape, lo, hi, dtype=jnp.int32)
    def uniform(self, shape, lo=0.0, hi=1.0):
        return jax.random.uniform(self._next(), shape, jnp.bfloat16, lo, hi)
    def permutation(self, n):
        return jax.random.permutation(self._next(), n)


kernel_name = 'interleave_layers__mha_block__dense_activation_mish__prompt'

def setup_inputs():
    _rng = _Rng(jax.random.key(int.from_bytes(__import__("os").urandom(4), "little")))
    _w = (lambda a: (lambda t: t.astype(jnp.bfloat16) if jnp.issubdtype(t.dtype, jnp.floating) else t)(jnp.asarray(a)))
    def _A_setup():
        B, S, D, H = 1, 2048, 512, 32
        return {
            "x": _w((lambda *s: _rng.normal(s) * 0.05)(B, S, D)),
            "wqkv": _w((lambda *s: _rng.normal(s) * 0.05)(D, 3 * D)),
            "wo": _w((lambda *s: _rng.normal(s) * 0.05)(D, D)),
        }
    _A_in = _A_setup()

    def _B_setup():
        B, S, D, F = 1, 2048, 512, 1792
        return {
            "x": _w((lambda *s: _rng.normal(s) * 0.05)(B, S, D)),
            "w1": _w((lambda *s: _rng.normal(s) * 0.4)(D, F) * (D ** -0.5)),
            "b1": _w((lambda *s: _rng.normal(s) * 0.4)(F)),
            "w2": _w((lambda *s: _rng.normal(s) * 0.4)(F, D) * (F ** -0.5)),
        }
    _B_in = _B_setup()

    return {
        "A_x": _A_in["x"],
        "A_wqkv": _A_in["wqkv"],
        "A_wo": _A_in["wo"],
        "B_x": _B_in["x"],
        "B_w1": _B_in["w1"],
        "B_b1": _B_in["b1"],
        "B_w2": _B_in["w2"],
    }

def reference(A_x, A_wqkv, A_wo, B_x, B_w1, B_b1, B_w2):
    def _A_ref(x, wqkv, wo):
        B, S, D = x.shape
        H = 32
        Dh = D // H
        qkv = (lambda x, *d: x.transpose(*d))((x @ wqkv).reshape(B, S, 3, H, Dh), 2, 0, 3, 1, 4)
        q, k, v = qkv[0], qkv[1], qkv[2]
        scores = jnp.einsum("bhqd,bhkd->bhqk", q, k) * (Dh ** -0.5)
        p = _softmax(scores, axis=-1)
        o = jnp.einsum("bhqk,bhkd->bhqd", p, v)
        return (lambda x, *d: x.transpose(*d))(o, 0, 2, 1, 3).reshape(B, S, D) @ wo

    def _B_ref(x, w1, b1, w2):
        h = jnp.einsum("bsd,df->bsf", x, w1) + b1
        sp = jnp.log1p(jnp.exp(-jnp.abs(h))) + jnp.where(h > 0, h, jnp.zeros_like(h))
        act = h * jnp.tanh(sp)
        return jnp.einsum("bsf,fd->bsd", act, w2)

    x = A_x
    x = x + _A_ref(_layernorm(x, axis=-1), A_wqkv, A_wo)
    x = x + _B_ref(_layernorm(x, axis=-1), B_w1, B_b1, B_w2)
    x = x + _A_ref(_layernorm(x, axis=-1), A_wqkv, A_wo)
    x = x + _B_ref(_layernorm(x, axis=-1), B_w1, B_b1, B_w2)
    return x
```

```python
import functools
import jax
import jax.numpy as jnp
from jax import lax
import jax.experimental.pallas as pl
import jax.experimental.pallas.tpu as pltpu

S, D, H, DH, F = 2048, 512, 32, 16, 1792
QW = 512
R = 128
TB = 512
LOG2E = 1.4426950408889634
QSCALE = (DH ** -0.5) * LOG2E
BF16, F32 = jnp.bfloat16, jnp.float32


def _tree(op, x, rows=8):
    while x.shape[0] > rows:
        h = x.shape[0] // 2
        x = op(x[:h], x[h:])
    return x


def _layernorm(x, eps=1e-5):
    m = jnp.mean(x, axis=-1, keepdims=True)
    d = x - m
    v = jnp.mean(d * d, axis=-1, keepdims=True)
    return d * lax.rsqrt(v + eps)


def _mish(h):
    t = jnp.exp(-jnp.abs(h))
    pos = h > 0
    n = jnp.where(pos, 1.0 + 2.0 * t, t * (t + 2.0))
    d = n + jnp.where(pos, 2.0 * t * t, 2.0)
    return h * n / d


def _kernel(x_hbm, wqkv_hbm, wo_hbm, w1_hbm, b1_hbm, w2_hbm, out_hbm,
            xin, wqkv, wo, w1, b1, w2, xres, ks, qts, vts, ots,
            g0, g1, s0, s1, m0, m1, obuf, sems, osems):
    NTB = S // TB
    x_cp = [pltpu.make_async_copy(x_hbm.at[pl.ds(t * TB, TB)], xin.at[pl.ds(t * TB, TB)], sems.at[t])
            for t in range(NTB)]
    wqkv_cp = pltpu.make_async_copy(wqkv_hbm, wqkv, sems.at[NTB])
    late = [pltpu.make_async_copy(src, dst, sems.at[NTB + 1 + i])
            for i, (src, dst) in enumerate(((wo_hbm, wo), (w1_hbm, w1), (b1_hbm, b1), (w2_hbm, w2)))]
    wqkv_cp.start()
    for c in x_cp:
        c.start()
    for c in late:
        c.start()

    gbuf, sbuf, mbuf = (g0, g1), (s0, s1), (m0, m1)
    row_head = lax.broadcasted_iota(jnp.int32, (128, QW), 0) // DH
    NU = S // R
    NITEM = (S // QW) * H

    def phase_a(t):
        rows = pl.ds(pl.multiple_of(t * TB, TB), TB)
        xn = _layernorm(xres[rows, :]).astype(BF16)
        q = jnp.dot(xn, wqkv[:, 0:D], preferred_element_type=F32)
        qts[:, rows] = (q * QSCALE).astype(BF16).T
        k = jnp.dot(xn, wqkv[:, D:2 * D], preferred_element_type=F32)
        ks[rows, :] = k.astype(BF16)
        v = jnp.dot(xn, wqkv[:, 2 * D:3 * D], preferred_element_type=F32)
        vts[:, rows] = v.astype(BF16).T

    def make_g(i, slot):
        h, qt = i % H, i // H
        g0_ = pl.multiple_of((h // 8) * 128, 128)
        q = qts[pl.ds(g0_, 128), pl.ds(pl.multiple_of(qt * QW, QW), QW)]
        gbuf[slot][...] = jnp.where(row_head == (h % 8), q, jnp.zeros_like(q))

    def p1(i, slot, rs, m):
        g0_ = pl.multiple_of(((i % H) // 8) * 128, 128)
        s = jnp.dot(ks[rs, pl.ds(g0_, 128)], gbuf[slot][...], preferred_element_type=F32)
        sbuf[slot][rs, :] = s
        return jnp.maximum(m, _tree(jnp.maximum, s))

    def p2(i, slot, rs, m, l, acc):
        v = vts[pl.ds(pl.multiple_of((i % H) * DH, DH), DH), rs]
        s = sbuf[slot][rs, :]
        p = jnp.exp2(s.reshape(R // 8, 8, QW) - m[None]).reshape(R, QW)
        l = l + _tree(jnp.add, p)
        acc = acc + jnp.dot(v, p.astype(BF16), preferred_element_type=F32)
        return l, acc

    def finish_max(m):
        return jnp.broadcast_to(jnp.max(m, axis=0, keepdims=True), (8, QW))

    def neg():
        return jnp.full((8, QW), -jnp.inf, F32)

    def step(i, cur):
        nxt = 1 - cur
        inext = jnp.minimum(i + 1, NITEM - 1)
        make_g(inext, nxt)
        m_cur = mbuf[cur][...]
        mn, l, acc = neg(), jnp.zeros((8, QW), F32), jnp.zeros((DH, QW), F32)
        for u in range(NU):
            rs = slice(u * R, (u + 1) * R)
            mn = p1(inext, nxt, rs, mn)
            l, acc = p2(i, cur, rs, m_cur, l, acc)
        mbuf[nxt][...] = finish_max(mn)
        o = acc / jnp.sum(l, axis=0, keepdims=True)
        ots[pl.ds(pl.multiple_of((i % H) * DH, DH), DH), pl.ds(pl.multiple_of((i // H) * QW, QW), QW)] = o.astype(BF16)

    def attention():
        make_g(0, 0)

        def b0(j, m):
            for u in range(4):
                m = p1(0, 0, pl.ds(pl.multiple_of(j * (R * 4) + u * R, R), R), m)
            return m
        m0[...] = finish_max(lax.fori_loop(0, NU // 4, b0, neg()))

        def body(i, c):
            @pl.when(i % 2 == 0)
            def _():
                step(i, 0)

            @pl.when(i % 2 == 1)
            def _():
                step(i, 1)
            return c
        lax.fori_loop(0, NITEM, body, 0)

    def phase_cd(t, last):
        rows = pl.ds(pl.multiple_of(t * TB, TB), TB)
        a = lax.dot_general(ots[:, rows], wo[...], (((0,), (0,)), ((), ())), preferred_element_type=F32)
        x1 = xres[rows, :] + a
        xn = _layernorm(x1).astype(BF16)
        h = jnp.dot(xn, w1[...], preferred_element_type=F32) + b1[...].astype(F32)
        act = _mish(h).astype(BF16)
        x2 = x1 + jnp.dot(act, w2[...], preferred_element_type=F32)

        @pl.when(jnp.logical_not(last))
        def _():
            xres[rows, :] = x2

        @pl.when(last)
        def _():
            obuf[rows, :] = x2.astype(BF16)
            pltpu.make_async_copy(obuf.at[rows], out_hbm.at[rows], osems.at[t]).start()

    wqkv_cp.wait()
    for t in range(NTB):
        x_cp[t].wait()
        xres[t * TB:(t + 1) * TB, :] = xin[t * TB:(t + 1) * TB, :].astype(F32)

    def layer(li, c):
        lax.fori_loop(0, NTB, lambda t, cc: (phase_a(t), cc)[1], 0)
        attention()

        @pl.when(li == 0)
        def _():
            for cp in late:
                cp.wait()
        lax.fori_loop(0, NTB, lambda t, cc: (phase_cd(t, li == 1), cc)[1], 0)
        return c
    lax.fori_loop(0, 2, layer, 0)
    for t in range(NTB):
        pltpu.make_async_copy(obuf.at[pl.ds(t * TB, TB)], out_hbm.at[pl.ds(t * TB, TB)], osems.at[t]).wait()


@jax.jit
def pallas_interleave_layers__mha_block__dense_activation_mish__prompt_kernel(A_x, A_wqkv, A_wo, B_x, B_w1, B_b1, B_w2):
    del B_x
    x = A_x.reshape(S, D)
    b1 = B_b1.reshape(1, F)
    any_spec = pl.BlockSpec(memory_space=pl.ANY)
    out = pl.pallas_call(
        _kernel,
        out_shape=jax.ShapeDtypeStruct((S, D), BF16),
        in_specs=[any_spec] * 6,
        out_specs=any_spec,
        scratch_shapes=[
            pltpu.VMEM((S, D), BF16), pltpu.VMEM((D, 3 * D), BF16), pltpu.VMEM((D, D), BF16),
            pltpu.VMEM((D, F), BF16), pltpu.VMEM((1, F), BF16), pltpu.VMEM((F, D), BF16),
            pltpu.VMEM((S, D), F32), pltpu.VMEM((S, D), BF16), pltpu.VMEM((D, S), BF16),
            pltpu.VMEM((D, S), BF16), pltpu.VMEM((D, S), BF16),
            pltpu.VMEM((128, QW), BF16), pltpu.VMEM((128, QW), BF16),
            pltpu.VMEM((S, QW), F32), pltpu.VMEM((S, QW), F32),
            pltpu.VMEM((8, QW), F32), pltpu.VMEM((8, QW), F32),
            pltpu.VMEM((S, D), BF16),
            pltpu.SemaphoreType.DMA((S // TB + 5,)), pltpu.SemaphoreType.DMA((S // TB,)),
        ],
        compiler_params=pltpu.CompilerParams(vmem_limit_bytes=110 * 1024 * 1024),
        name="fused_mha_mish_2layer",
    )(x, A_wqkv, A_wo, B_w1, b1, B_w2)
    return out.reshape(1, S, D)
```

```python
import jax
import jax.numpy as jnp
from jax import lax
import jax.experimental.pallas as pl
import jax.experimental.pallas.tpu as pltpu

S, D, H, DH, F = 2048, 512, 32, 16, 1792
QW = 512
R = 128
NC = QW // 128
NU = S // R
HG = 128 // DH
NG = H // HG
NBLK = (S // QW) * NG
TB = 512
NTB = S // TB
SUB = 4
LOG2E = 1.4426950408889634
QSCALE = (DH ** -0.5) * LOG2E
BF16, F32, U32 = jnp.bfloat16, jnp.float32, jnp.uint32


def _bf(x):
    return pltpu.bitcast(x, BF16)


def _u32(x):
    return pltpu.bitcast(x, U32)


def _tree(op, x):
    while x.shape[0] > 8:
        h = x.shape[0] // 2
        x = op(x[:h], x[h:])
    return x


def _fold_max(init, x):
    return jnp.maximum(init, _tree(jnp.maximum, x))


def _fold_sum(init, x):
    for j in range(0, x.shape[0] // 8, 4):
        y = x[j * 8:(j + 4) * 8]
        init = init + ((y[0:8] + y[8:16]) + (y[16:24] + y[24:32]))
    return init


def _layernorm(x, eps=1e-5):
    m = jnp.mean(x, axis=-1, keepdims=True)
    d = x - m
    v = jnp.mean(d * d, axis=-1, keepdims=True)
    return d * lax.rsqrt(v + eps)


def _recip(d):
    r = pl.reciprocal(d, approx=True)
    return r * (2.0 - d * r)


def _mish(h):
    e = jnp.exp(jnp.minimum(h, 20.0))
    n = e * (e + 2.0)
    return (h * n) * _recip(n + 2.0)


def _kernel(x_hbm, wqkv_hbm, wo_hbm, w1_hbm, b1_hbm, w2_hbm, out_hbm,
            xin, wqkv, wo, w1, b1, w2, xres, ks, qs, vs, ots,
            s0, s1, m0, obuf, xnb, sems, osems):
    def x_copy(t):
        rows = pl.ds(pl.multiple_of(t * TB, TB), TB)
        return pltpu.make_async_copy(x_hbm.at[rows], xin.at[rows], sems.at[t])

    wqkv_cp = pltpu.make_async_copy(wqkv_hbm, wqkv, sems.at[NTB])
    late = [pltpu.make_async_copy(src, dst, sems.at[NTB + 1 + i])
            for i, (src, dst) in enumerate(((wo_hbm, wo), (w1_hbm, w1), (b1_hbm, b1), (w2_hbm, w2)))]
    x_copy(0).start()
    wqkv_cp.start()

    sbuf = (s0, s1)

    def load_ln(t, li):
        rows = pl.ds(pl.multiple_of(t * TB, TB), TB)
        x = jnp.where(li == 0, xin[rows, :].astype(F32), xres[rows, :])
        xres[rows, :] = x
        return _layernorm(x).astype(BF16)

    def qkv_matmuls(t, xn):
        r0 = pl.multiple_of(t * TB, TB)
        q = jnp.dot(xn, wqkv[:, 0:D], preferred_element_type=F32)
        qt = _u32((q * QSCALE).astype(BF16).T)
        for c in range(TB // 128):
            qs[t * (TB // 128) + c] = qt[:, c * 128:(c + 1) * 128]
        v = jnp.dot(xn, wqkv[:, 2 * D:3 * D], preferred_element_type=F32)
        vt = _u32(v.astype(BF16).T)
        for c in range(TB // 128):
            vs[t * (TB // 128) + c] = vt[:, c * 128:(c + 1) * 128]
        k = _u32(jnp.dot(xn, wqkv[:, D:2 * D], preferred_element_type=F32).astype(BF16))
        for g in range(NG):
            ks[g, pl.ds(pl.multiple_of(r0 // 2, TB // 2), TB // 2), :] = k[:, g * 128:(g + 1) * 128]

    def phase_a(li):
        @pl.when(li == 0)
        def _():
            x_copy(0).wait()
            x_copy(1).start()
        xnb[0:TB // 2, :] = _u32(load_ln(0, li))

        @pl.when(li == 0)
        def _():
            wqkv_cp.wait()
            for t in range(2, NTB):
                x_copy(t).start()
            for c in late:
                c.start()

        def body(t, carry):
            tn = jnp.minimum(t + 1, NTB - 1)

            @pl.when(jnp.logical_and(li == 0, t + 1 < NTB))
            def _():
                x_copy(tn).wait()
            r0 = pl.multiple_of(t * (TB // 2), TB // 2)
            qkv_matmuls(t, _bf(xnb[pl.ds(r0, TB // 2), :]))
            xn_next = load_ln(tn, li)
            xnb[pl.ds(pl.multiple_of(tn * (TB // 2), TB // 2), TB // 2), :] = _u32(xn_next)
            return carry
        lax.fori_loop(0, NTB, body, 0)

    def g_tile(qt, g, j, c):
        q = qs[qt * NC + c, pl.ds(pl.multiple_of(g * 64 + 8 * j, 8), 8), :]
        parts = []
        if j > 0:
            parts.append(jnp.zeros((8 * j, 128), U32))
        parts.append(q)
        if j < HG - 1:
            parts.append(jnp.zeros((56 - 8 * j, 128), U32))
        return _bf(jnp.concatenate(parts, axis=0))

    def pass1(qt, g, j, slot, u, c, mc, kk):
        s = jnp.dot(kk, g_tile(qt, g, j, c), preferred_element_type=F32)
        sbuf[slot][u * R:(u + 1) * R, c * 128:(c + 1) * 128] = s
        return _fold_max(mc, s)

    def pass2(slot, u, c, mc, lc, ac, v):
        s = sbuf[slot][u * R:(u + 1) * R, c * 128:(c + 1) * 128]
        z = (s.reshape(R // 8, 8, 128) - mc[None]).reshape(R, 128)
        p = jnp.exp2(z)
        lc = _fold_sum(lc, p)
        ac = ac + jnp.dot(v, p.astype(BF16), preferred_element_type=F32)
        return lc, ac

    def fin_max(m):
        return jnp.broadcast_to(jnp.max(m, axis=0, keepdims=True), (8, 128))

    def neg_inf():
        return [jnp.full((8, 128), -jnp.inf, F32) for _ in range(NC)]

    def write_o(qt, g, j, l, acc):
        for c in range(NC):
            o = acc[c] * _recip(jnp.sum(l[c], axis=0, keepdims=True))
            ots[pl.ds(pl.multiple_of(g * 64 + 8 * j, 8), 8),
                pl.ds(pl.multiple_of(qt * QW + c * 128, 128), 128)] = _u32(o.astype(BF16))

    def attn_block(b, m_first, last_block):
        qt, g = b // NG, b % NG
        bn = b + 1 if last_block else jnp.minimum(b + 1, NBLK - 1)
        qtn, gn = bn // NG, bn % NG
        mn = {j: neg_inf() for j in range(1, HG + 1)}
        mcur = {0: m_first}
        l = [jnp.zeros((8, 128), F32) for _ in range(NC)]
        acc = [jnp.zeros((DH, 128), F32) for _ in range(NC)]
        hist = {}
        tot = HG * NU
        for gi in range(tot + 1):
            if gi < tot:
                j, u = gi // NU, gi % NU
                if not (last_block and j == HG - 1):
                    a_qt, a_g, a_j = (qt, g, j + 1) if j < HG - 1 else (qtn, gn, 0)
                    kk = _bf(ks[a_g, u * (R // 2):(u + 1) * (R // 2), :])
                    for c in range(NC):
                        mn[j + 1][c] = pass1(a_qt, a_g, a_j, (j + 1) % 2, u, c, mn[j + 1][c], kk)
                    hist[gi] = list(mn[j + 1])
                    if u == NU - 1:
                        mcur[j + 1] = [fin_max(x) for x in mn[j + 1]]
            g2 = gi - 1
            if g2 >= 0:
                j, u = g2 // NU, g2 % NU
                v = _bf(vs[u, pl.ds(pl.multiple_of(g * 64 + 8 * j, 8), 8), :])
                for c in range(NC):
                    mu = mcur[j][c]
                    if (g2 - 2) in hist:
                        ref = hist[g2 - 2][c]
                        mu = jnp.where(ref > jnp.inf, ref, mu)
                    l[c], acc[c] = pass2(j % 2, u, c, mu, l[c], acc[c], v)
                if u == NU - 1:
                    write_o(qt, g, j, l, acc)
                    l = [jnp.zeros((8, 128), F32) for _ in range(NC)]
                    acc = [jnp.zeros((DH, 128), F32) for _ in range(NC)]
        return mcur.get(HG)

    def attention():
        m = neg_inf()
        for u in range(NU):
            kk = _bf(ks[0, u * (R // 2):(u + 1) * (R // 2), :])
            for c in range(NC):
                m[c] = pass1(0, 0, 0, 0, u, c, m[c], kk)
        for c in range(NC):
            m0[:, c * 128:(c + 1) * 128] = fin_max(m[c])

        def body(b, carry):
            mo = attn_block(b, [m0[:, c * 128:(c + 1) * 128] for c in range(NC)], False)
            for c in range(NC):
                m0[:, c * 128:(c + 1) * 128] = mo[c]
            return carry
        lax.fori_loop(0, NBLK - 1, body, 0)
        attn_block(NBLK - 1, [m0[:, c * 128:(c + 1) * 128] for c in range(NC)], True)

    def phase_cd(t, last):
        r0 = pl.multiple_of(t * TB, TB)
        RS = TB // SUB
        b1v = b1[...].astype(F32).reshape(1, F)
        rws = [pl.ds(pl.multiple_of(r0 + j * RS, RS), RS) for j in range(SUB)]
        x1, xn, act = [], [], []
        for j in range(SUB):
            ot = _bf(ots[:, rws[j]])
            a = lax.dot_general(ot, wo[...], (((0,), (0,)), ((), ())), preferred_element_type=F32)
            x1.append(xres[rws[j], :] + a)
            xn.append(_layernorm(x1[j]).astype(BF16))
        for j in range(SUB):
            h = jnp.dot(xn[j], w1[...], preferred_element_type=F32) + b1v
            act.append(_mish(h).astype(BF16))
        for j in range(SUB):
            x2 = x1[j] + jnp.dot(act[j], w2[...], preferred_element_type=F32)
            xres[rws[j], :] = x2
            obuf[rws[j], :] = x2.astype(BF16)

        @pl.when(last)
        def _():
            out_copy(t).start()

    def out_copy(t):
        rows = pl.ds(pl.multiple_of(t * TB, TB), TB)
        return pltpu.make_async_copy(obuf.at[rows], out_hbm.at[rows], osems.at[t])

    def layer(li, carry):
        phase_a(li)
        attention()

        @pl.when(li == 0)
        def _():
            for cp in late:
                cp.wait()

        def cd_body(t, c):
            phase_cd(t, li == 1)
            return c
        lax.fori_loop(0, NTB, cd_body, 0)
        return carry
    lax.fori_loop(0, 2, layer, 0)
    for t in range(NTB):
        out_copy(t).wait()


@jax.jit
def pallas_interleave_layers__mha_block__dense_activation_mish__prompt_kernel(
    A_x: jax.Array,
    A_wqkv: jax.Array,
    A_wo: jax.Array,
    B_x: jax.Array,
    B_w1: jax.Array,
    B_b1: jax.Array,
    B_w2: jax.Array,
):
    del B_x
    any_spec = pl.BlockSpec(memory_space=pl.ANY)
    out = pl.pallas_call(
        _kernel,
        out_shape=jax.ShapeDtypeStruct((S, D), BF16),
        in_specs=[any_spec] * 6,
        out_specs=any_spec,
        scratch_shapes=[
            pltpu.VMEM((S, D), BF16),
            pltpu.VMEM((D, 3 * D), BF16),
            pltpu.VMEM((D, D), BF16),
            pltpu.VMEM((D, F), BF16),
            pltpu.VMEM((F,), BF16),
            pltpu.VMEM((F, D), BF16),
            pltpu.VMEM((S, D), F32),
            pltpu.VMEM((NG, S // 2, 128), U32),
            pltpu.VMEM((S // 128, D // 2, 128), U32),
            pltpu.VMEM((S // 128, D // 2, 128), U32),
            pltpu.VMEM((D // 2, S), U32),
            pltpu.VMEM((S, QW), F32),
            pltpu.VMEM((S, QW), F32),
            pltpu.VMEM((8, QW), F32),
            pltpu.VMEM((S, D), BF16),
            pltpu.VMEM((S // 2, D), U32),
            pltpu.SemaphoreType.DMA((NTB + 5,)),
            pltpu.SemaphoreType.DMA((NTB,)),
        ],
        compiler_params=pltpu.CompilerParams(vmem_limit_bytes=110 * 1024 * 1024),
        name="fused_mha_mish_2layer",
    )(A_x.reshape(S, D), A_wqkv, A_wo, B_w1, B_b1, B_w2)
    return out.reshape(1, S, D)
```

```python
import jax
import jax.numpy as jnp
from jax import lax
import jax.experimental.pallas as pl
import jax.experimental.pallas.tpu as pltpu

S, D, H, DH, F = 2048, 512, 32, 16, 1792
QW = 512
R = 128
NC = QW // 128
NU = S // R
HG = 128 // DH
NG = H // HG
NBLK = (S // QW) * NG
TB = 512
NTB = S // TB
SUB = 4
LOG2E = 1.4426950408889634
QSCALE = (DH ** -0.5) * LOG2E
BF16, F32, U32 = jnp.bfloat16, jnp.float32, jnp.uint32


def _bf(x):
    return pltpu.bitcast(x, BF16)


def _u32(x):
    return pltpu.bitcast(x, U32)


def _tree(op, x):
    while x.shape[0] > 8:
        h = x.shape[0] // 2
        x = op(x[:h], x[h:])
    return x


def _fold_max(init, x):
    return jnp.maximum(init, _tree(jnp.maximum, x))


def _fold_sum(init, x):
    for j in range(0, x.shape[0] // 8, 4):
        y = x[j * 8:(j + 4) * 8]
        init = init + ((y[0:8] + y[8:16]) + (y[16:24] + y[24:32]))
    return init


def _layernorm(x, eps=1e-5):
    m = jnp.mean(x, axis=-1, keepdims=True)
    d = x - m
    v = jnp.mean(d * d, axis=-1, keepdims=True)
    return d * lax.rsqrt(v + eps)


def _recip(d):
    r = pl.reciprocal(d, approx=True)
    return r * (2.0 - d * r)


def _mish(h):
    e = jnp.exp(jnp.minimum(h, 20.0))
    n = e * (e + 2.0)
    return (h * n) * _recip(n + 2.0)


def _kernel(x_hbm, wqkv_hbm, wo_hbm, w1_hbm, b1_hbm, w2_hbm, out_hbm,
            xin, wqkv, wo, w1, b1, w2, xres, ks, qs, vs, ots,
            s0, s1, m0, obuf, xnb, sems, osems, wsems):
    def x_copy(t):
        rows = pl.ds(pl.multiple_of(t * TB, TB), TB)
        return pltpu.make_async_copy(x_hbm.at[rows], xin.at[rows], sems.at[t])

    def wcol_copy(j):
        return pltpu.make_async_copy(wqkv_hbm.at[:, pl.ds(j * D, D)], wqkv.at[:, pl.ds(j * D, D)], wsems.at[j])

    late = [pltpu.make_async_copy(src, dst, sems.at[NTB + i])
            for i, (src, dst) in enumerate(((wo_hbm, wo), (w1_hbm, w1), (b1_hbm, b1), (w2_hbm, w2)))]
    x_copy(0).start()
    wcol_copy(0).start()

    sbuf = (s0, s1)

    def zero_rows(i, carry):
        xres[pl.ds(pl.multiple_of(2 * TB + i * 128, 128), 128), :] = jnp.zeros((128, D), F32)
        return carry
    lax.fori_loop(0, (S - 2 * TB) // 128, zero_rows, 0)

    def load_ln(t, li):
        rows = pl.ds(pl.multiple_of(t * TB, TB), TB)
        x = jnp.where(li == 0, xin[rows, :].astype(F32), xres[rows, :])
        xres[rows, :] = x
        return _layernorm(x).astype(BF16)

    def qkv_matmuls(t, xn, hooks=None):
        r0 = pl.multiple_of(t * TB, TB)
        if hooks:
            hooks[0]()
        q = jnp.dot(xn, wqkv[:, 0:D], preferred_element_type=F32)
        qt = _u32((q * QSCALE).astype(BF16).T)
        for c in range(TB // 128):
            qs[t * (TB // 128) + c] = qt[:, c * 128:(c + 1) * 128]
        if hooks:
            hooks[1]()
        v = jnp.dot(xn, wqkv[:, 2 * D:3 * D], preferred_element_type=F32)
        vt = _u32(v.astype(BF16).T)
        for c in range(TB // 128):
            vs[t * (TB // 128) + c] = vt[:, c * 128:(c + 1) * 128]
        if hooks:
            hooks[2]()
        k = _u32(jnp.dot(xn, wqkv[:, D:2 * D], preferred_element_type=F32).astype(BF16))
        for g in range(NG):
            ks[g, pl.ds(pl.multiple_of(r0 // 2, TB // 2), TB // 2), :] = k[:, g * 128:(g + 1) * 128]

    def first_block():
        x_copy(0).wait()
        wcol_copy(2).start()
        x = xin[0:TB, :].astype(F32)
        xres[0:TB, :] = x
        xn = _layernorm(x).astype(BF16)

        def h0():
            wcol_copy(0).wait()
            wcol_copy(1).start()

        def h1():
            wcol_copy(2).wait()
            x_copy(1).start()

        def h2():
            wcol_copy(1).wait()
        qkv_matmuls(0, xn, (h0, h1, h2))
        x_copy(1).wait()
        for t in range(2, NTB):
            x_copy(t).start()
        for c in late:
            c.start()
        x = xin[TB:2 * TB, :].astype(F32)
        xres[TB:2 * TB, :] = x
        xnb[TB // 2:TB, :] = _u32(_layernorm(x).astype(BF16))

    def phase_a(li):
        @pl.when(li != 0)
        def _():
            xnb[0:TB // 2, :] = _u32(_layernorm(xres[0:TB, :]).astype(BF16))

        def body(t, carry):
            tn = jnp.minimum(t + 1, NTB - 1)

            @pl.when(jnp.logical_and(li == 0, t + 1 < NTB))
            def _():
                x_copy(tn).wait()
            r0 = pl.multiple_of(t * (TB // 2), TB // 2)
            qkv_matmuls(t, _bf(xnb[pl.ds(r0, TB // 2), :]))
            xn_next = load_ln(tn, li)
            xnb[pl.ds(pl.multiple_of(tn * (TB // 2), TB // 2), TB // 2), :] = _u32(xn_next)
            return carry
        lax.fori_loop(jnp.where(li == 0, 1, 0), NTB, body, 0)

    def g_tile(qt, g, j, c):
        q = qs[qt * NC + c, pl.ds(pl.multiple_of(g * 64 + 8 * j, 8), 8), :]
        parts = []
        if j > 0:
            parts.append(jnp.zeros((8 * j, 128), U32))
        parts.append(q)
        if j < HG - 1:
            parts.append(jnp.zeros((56 - 8 * j, 128), U32))
        return _bf(jnp.concatenate(parts, axis=0))

    def pass1(qt, g, j, slot, u, c, mc, kk):
        s = jnp.dot(kk, g_tile(qt, g, j, c), preferred_element_type=F32)
        sbuf[slot][u * R:(u + 1) * R, c * 128:(c + 1) * 128] = s
        return _fold_max(mc, s)

    def pass2(slot, u, c, mc, lc, ac, v):
        s = sbuf[slot][u * R:(u + 1) * R, c * 128:(c + 1) * 128]
        z = (s.reshape(R // 8, 8, 128) - mc[None]).reshape(R, 128)
        p = jnp.exp2(z)
        lc = _fold_sum(lc, p)
        ac = ac + jnp.dot(v, p.astype(BF16), preferred_element_type=F32)
        return lc, ac

    def fin_max(m):
        return jnp.broadcast_to(jnp.max(m, axis=0, keepdims=True), (8, 128))

    def neg_inf():
        return [jnp.full((8, 128), -jnp.inf, F32) for _ in range(NC)]

    def write_o(qt, g, j, l, acc):
        for c in range(NC):
            o = acc[c] * _recip(jnp.sum(l[c], axis=0, keepdims=True))
            ots[pl.ds(pl.multiple_of(g * 64 + 8 * j, 8), 8),
                pl.ds(pl.multiple_of(qt * QW + c * 128, 128), 128)] = _u32(o.astype(BF16))

    def attn_block(b, m_first, last_block):
        qt, g = b // NG, b % NG
        bn = b + 1 if last_block else jnp.minimum(b + 1, NBLK - 1)
        qtn, gn = bn // NG, bn % NG
        mn = {j: neg_inf() for j in range(1, HG + 1)}
        mcur = {0: m_first}
        l = [jnp.zeros((8, 128), F32) for _ in range(NC)]
        acc = [jnp.zeros((DH, 128), F32) for _ in range(NC)]
        hist = {}
        tot = HG * NU
        for gi in range(tot + 1):
            if gi < tot:
                j, u = gi // NU, gi % NU
                if not (last_block and j == HG - 1):
                    a_qt, a_g, a_j = (qt, g, j + 1) if j < HG - 1 else (qtn, gn, 0)
                    kk = _bf(ks[a_g, u * (R // 2):(u + 1) * (R // 2), :])
                    for c in range(NC):
                        mn[j + 1][c] = pass1(a_qt, a_g, a_j, (j + 1) % 2, u, c, mn[j + 1][c], kk)
                    hist[gi] = list(mn[j + 1])
                    if u == NU - 1:
                        mcur[j + 1] = [fin_max(x) for x in mn[j + 1]]
            g2 = gi - 1
            if g2 >= 0:
                j, u = g2 // NU, g2 % NU
                v = _bf(vs[u, pl.ds(pl.multiple_of(g * 64 + 8 * j, 8), 8), :])
                for c in range(NC):
                    mu = mcur[j][c]
                    if (g2 - 2) in hist:
                        ref = hist[g2 - 2][c]
                        mu = jnp.where(ref > jnp.inf, ref, mu)
                    l[c], acc[c] = pass2(j % 2, u, c, mu, l[c], acc[c], v)
                if u == NU - 1:
                    write_o(qt, g, j, l, acc)
                    l = [jnp.zeros((8, 128), F32) for _ in range(NC)]
                    acc = [jnp.zeros((DH, 128), F32) for _ in range(NC)]
        return mcur.get(HG)

    def attention():
        m = neg_inf()
        for u in range(NU):
            kk = _bf(ks[0, u * (R // 2):(u + 1) * (R // 2), :])
            for c in range(NC):
                m[c] = pass1(0, 0, 0, 0, u, c, m[c], kk)
        for c in range(NC):
            m0[:, c * 128:(c + 1) * 128] = fin_max(m[c])

        def body(b, carry):
            mo = attn_block(b, [m0[:, c * 128:(c + 1) * 128] for c in range(NC)], False)
            for c in range(NC):
                m0[:, c * 128:(c + 1) * 128] = mo[c]
            return carry
        lax.fori_loop(0, NBLK - 1, body, 0)
        attn_block(NBLK - 1, [m0[:, c * 128:(c + 1) * 128] for c in range(NC)], True)

    def phase_cd(t, last):
        r0 = pl.multiple_of(t * TB, TB)
        RS = TB // SUB
        b1v = b1[...].astype(F32).reshape(1, F)
        rws = [pl.ds(pl.multiple_of(r0 + j * RS, RS), RS) for j in range(SUB)]
        x1, xn, act = [], [], []
        for j in range(SUB):
            ot = _bf(ots[:, rws[j]])
            a = lax.dot_general(ot, wo[...], (((0,), (0,)), ((), ())), preferred_element_type=F32)
            x1.append(xres[rws[j], :] + a)
            xn.append(_layernorm(x1[j]).astype(BF16))
        for j in range(SUB):
            h = jnp.dot(xn[j], w1[...], preferred_element_type=F32) + b1v
            act.append(_mish(h).astype(BF16))
        for j in range(SUB):
            x2 = x1[j] + jnp.dot(act[j], w2[...], preferred_element_type=F32)
            xres[rws[j], :] = x2
            obuf[rws[j], :] = x2.astype(BF16)

        @pl.when(last)
        def _():
            out_copy(t).start()

    def out_copy(t):
        rows = pl.ds(pl.multiple_of(t * TB, TB), TB)
        return pltpu.make_async_copy(obuf.at[rows], out_hbm.at[rows], osems.at[t])

    def layer(li, carry):
        phase_a(li)
        attention()

        @pl.when(li == 0)
        def _():
            for cp in late:
                cp.wait()

        def cd_body(t, c):
            phase_cd(t, li == 1)
            return c
        lax.fori_loop(0, NTB, cd_body, 0)
        return carry
    first_block()
    lax.fori_loop(0, 2, layer, 0)
    for t in range(NTB):
        out_copy(t).wait()


@jax.jit
def pallas_interleave_layers__mha_block__dense_activation_mish__prompt_kernel(
    A_x: jax.Array,
    A_wqkv: jax.Array,
    A_wo: jax.Array,
    B_x: jax.Array,
    B_w1: jax.Array,
    B_b1: jax.Array,
    B_w2: jax.Array,
):
    del B_x
    any_spec = pl.BlockSpec(memory_space=pl.ANY)
    out = pl.pallas_call(
        _kernel,
        out_shape=jax.ShapeDtypeStruct((S, D), BF16),
        in_specs=[any_spec] * 6,
        out_specs=any_spec,
        scratch_shapes=[
            pltpu.VMEM((S, D), BF16),
            pltpu.VMEM((D, 3 * D), BF16),
            pltpu.VMEM((D, D), BF16),
            pltpu.VMEM((D, F), BF16),
            pltpu.VMEM((F,), BF16),
            pltpu.VMEM((F, D), BF16),
            pltpu.VMEM((S, D), F32),
            pltpu.VMEM((NG, S // 2, 128), U32),
            pltpu.VMEM((S // 128, D // 2, 128), U32),
            pltpu.VMEM((S // 128, D // 2, 128), U32),
            pltpu.VMEM((D // 2, S), U32),
            pltpu.VMEM((S, QW), F32),
            pltpu.VMEM((S, QW), F32),
            pltpu.VMEM((8, QW), F32),
            pltpu.VMEM((S, D), BF16),
            pltpu.VMEM((S // 2, D), U32),
            pltpu.SemaphoreType.DMA((NTB + 4,)),
            pltpu.SemaphoreType.DMA((NTB,)),
            pltpu.SemaphoreType.DMA((3,)),
        ],
        compiler_params=pltpu.CompilerParams(vmem_limit_bytes=110 * 1024 * 1024),
        name="fused_mha_mish_2layer",
    )(A_x.reshape(S, D), A_wqkv, A_wo, B_w1, B_b1, B_w2)
    return out.reshape(1, S, D)
```
